```python
import os as _os
_os.environ.setdefault("JAX_PLATFORMS", "cpu")
import jax
import jax.numpy as jnp

def _softmax(x, axis=-1):
    return jax.nn.softmax(x, axis=axis)
def _gelu(x):
    return jax.nn.gelu(x, approximate=True)
def _silu(x):
    return jax.nn.silu(x)
def _sigmoid(x):
    return jax.nn.sigmoid(x)
def _layernorm(x, axis=-1, eps=1e-5):
    m = jnp.mean(x, axis=axis, keepdims=True)
    v = jnp.var(x, axis=axis, keepdims=True)
    return (x - m) / jnp.sqrt(v + eps)
def _scatter_add(tgt, idx, src, axis=0):
    return tgt.at[idx].add(src)
def _segment_sum(src, seg, n):
    return jax.ops.segment_sum(src, seg, n)
class _Rng:
    def __init__(self, key):
        self._k = key
    def _next(self):
        self._k, sub = jax.random.split(self._k)
        return sub
    def normal(self, shape):
        return jax.random.normal(self._next(), shape, dtype=jnp.bfloat16)
    def randint(self, lo, hi, shape):
        return jax.random.randint(self._next(), shape, lo, hi, dtype=jnp.int32)
    def uniform(self, shape, lo=0.0, hi=1.0):
        return jax.random.uniform(self._next(), shape, jnp.bfloat16, lo, hi)
    def permutation(self, n):
        return jax.random.permutation(self._next(), n)


kernel_name = 'gated_mix__compressed_kv_cla__linear_attn_block__prompt'

def setup_inputs():
    _rng = _Rng(jax.random.key(int.from_bytes(__import__("os").urandom(4), "little")))
    _w = (lambda a: (lambda t: t.astype(jnp.bfloat16) if jnp.issubdtype(t.dtype, jnp.floating) else t)(jnp.asarray(a)))
    def _A_setup():
        B, H, Sq, Sk, D, M = 1, 16, 2048, 2048, 256, 448
        Dc = 4 * D
        return {
            "x": _w((lambda *s: _rng.normal(s) * 0.05)(B, Sq, M)),
            "c_kv": _w((lambda *s: _rng.normal(s) * 0.8)(B, Sk, Dc)),
            "w_q": _w((lambda *s: _rng.normal(s) * 3.2)(M, H, D) * (M ** -0.5)),
            "w_uk": _w((lambda *s: _rng.normal(s) * 3.2)(Dc, H, D) * (Dc ** -0.5)),
            "w_uv": _w((lambda *s: _rng.normal(s) * 0.8)(Dc, H, D) * (Dc ** -0.5)),
            "w_o": _w((lambda *s: _rng.normal(s) * 0.8)(H, D, M) * ((H * D) ** -0.5)),
        }
    _A_in = _A_setup()

    def _B_setup():
        B, S, D = 1, 2048, 448
        return {
            "x": _w((lambda *s: _rng.normal(s) * 0.05)(B, S, D)),
            "wqkv": _w((lambda *s: _rng.normal(s) * 1.6)(D, 3 * D)),
            "wo": _w((lambda *s: _rng.normal(s) * 0.4)(D, D)),
        }
    _B_in = _B_setup()

    return {
        "A_x": _A_in["x"],
        "A_c_kv": _A_in["c_kv"],
        "A_w_q": _A_in["w_q"],
        "A_w_uk": _A_in["w_uk"],
        "A_w_uv": _A_in["w_uv"],
        "A_w_o": _A_in["w_o"],
        "B_x": _B_in["x"],
        "B_wqkv": _B_in["wqkv"],
        "B_wo": _B_in["wo"],
        "gate_w": _w((lambda *s: _rng.normal(s) * 0.05)(448) * 16.0),
    }

def reference(A_x, A_c_kv, A_w_q, A_w_uk, A_w_uv, A_w_o, B_x, B_wqkv, B_wo, gate_w):
    def _A_ref(x, c_kv, w_q, w_uk, w_uv, w_o):
        B, Sq, M = x.shape[0], x.shape[1], x.shape[2]
        Sk = c_kv.shape[1]
        H, D = w_q.shape[1], w_q.shape[2]
        q = jnp.einsum("bqm,mhd->bhqd", x, w_q)
        k = jnp.einsum("bkc,chd->bhkd", c_kv, w_uk)
        v = jnp.einsum("bkc,chd->bhkd", c_kv, w_uv)
        scores = jnp.einsum("bhqd,bhkd->bhqk", q, k) * (D ** -0.5)
        off = Sk - Sq
        qi = jnp.arange(Sq)[:, None]
        kj = jnp.arange(Sk)[None, :]
        cmask = kj <= (qi + off)
        scores = jnp.where(cmask[None, None], scores, -1e9)
        p = _softmax(scores, axis=-1)
        ctx = jnp.einsum("bhqk,bhkd->bhqd", p, v)
        return jnp.einsum("bhqd,hdm->bqm", ctx, w_o)

    def _B_ref(x, wqkv, wo):
        B, S, D = x.shape
        H = 16; Dh = D // H
        qkv = (lambda x, *d: x.transpose(*d))((x @ wqkv).reshape(B, S, 3, H, Dh), 2, 0, 3, 1, 4)
        q, k, v = qkv[0], qkv[1], qkv[2]
        phi = lambda t: jnp.where(t > 0, t + 1, jnp.exp(t)) + 1e-6
        pq, pk = phi(q), phi(k)
        kv = jnp.einsum("bhsd,bhse->bhde", pk, v)
        z = jnp.einsum("bhsd->bhd", pk)
        num = jnp.einsum("bhqd,bhde->bhqe", pq, kv)
        den = jnp.einsum("bhqd,bhd->bhq", pq, z)[..., None] + 1e-6
        o = num / den
        return (lambda x, *d: x.transpose(*d))(o, 0, 2, 1, 3).reshape(B, S, D) @ wo

    x = A_x
    g = _sigmoid((x * gate_w).sum(-1, keepdims=True))
    a = _A_ref(x, A_c_kv, A_w_q, A_w_uk, A_w_uv, A_w_o)
    b = _B_ref(x, B_wqkv, B_wo)
    return g * a + (1 - g) * b
```

```python
import jax
import jax.numpy as jnp
from jax import lax
from jax.experimental import pallas as pl
from jax.experimental.pallas import tpu as pltpu

S = 2048
M = 448
H = 16
D = 256
DC = 1024
DH = 28
G = 4
GW = 112
BQ = 256
HB = BQ // 2
NB = S // BQ
NX = 4
XC = S // NX
LOOK = 2
ORDER = (7, 0, 6, 1, 5, 2, 4, 3)
LOG2E = 1.4426950408889634
MASKED = -1e9 * LOG2E
F32 = jnp.float32
BF16 = jnp.bfloat16
U32 = jnp.uint32
NT = (((1,), (1,)), ((), ()))


def _dot(a, b):
    return jnp.dot(a, b, preferred_element_type=F32)


def _dot_nt(a, b):
    return lax.dot_general(a, b, NT, preferred_element_type=F32)


def _half(w, hi):
    w = (w & U32(0xFFFF0000)) if hi else (w << 16)
    return pltpu.bitcast(w, F32).astype(BF16)


def _ld(ref, pre, r0, r1):
    return pltpu.bitcast(ref[pre + (slice(r0 // 2, r1 // 2), slice(None))], BF16)


def _st(ref, pre, r0, r1, val):
    ref[pre + (slice(r0 // 2, r1 // 2), slice(None))] = pltpu.bitcast(val, U32)


def _phi(t):
    return jnp.where(t > 0, t + 1.0, jnp.exp(t)) + 1e-6


def _kernel(xt_hbm, c_hbm, wq_hbm, wk_hbm, wv_hbm, wot_hbm, wqkv_hbm, bwo_hbm, gw_ref,
            out_hbm,
            xt_s, x_s, c_s, wq_s, wk_s, wv_s, wot_s, wqkv_s, bwo_s,
            q_s, k_s, v_s, ctx_s, bt_s, g_s, out_s, sem, wsem, osem):
    wts = ((wq_hbm, wq_s), (wk_hbm, wk_s), (wv_hbm, wv_s))

    def wcopies(j):
        return [pltpu.make_async_copy(src.bitcast(U32).at[:, j, :], dst.at[j], wsem.at[m * (H // 2) + j])
                for m, (src, dst) in enumerate(wts)]

    def wqkv_cols(c0, c1, n):
        return pltpu.make_async_copy(wqkv_hbm.at[:, pl.ds(c0, c1 - c0)],
                                     wqkv_s.at[:, pl.ds(c0, c1 - c0)], sem.at[n])

    cp_wa = wqkv_cols(384, 896, 0)
    cp_wb = [wqkv_cols(0, 384, 1), wqkv_cols(896, 3 * M, 2),
             pltpu.make_async_copy(bwo_hbm, bwo_s, sem.at[3])]
    cp_c = pltpu.make_async_copy(c_hbm.bitcast(U32), c_s, sem.at[4])
    cp_wot = pltpu.make_async_copy(wot_hbm.bitcast(U32), wot_s, sem.at[5])
    cp_xt = [pltpu.make_async_copy(xt_hbm.bitcast(U32).at[:, pl.ds(n * XC, XC)],
                                   xt_s.at[:, pl.ds(n * XC, XC)], sem.at[6 + n]) for n in range(NX)]

    cp_wa.start()
    cp_xt[0].start()
    cp_wa.wait()
    wtk = wqkv_s[:, 384:896].T[64:]
    pks = []
    for n in range(NX):
        if n + 1 < NX:
            cp_xt[n + 1].start()
        if n == 0:
            for cp in cp_wb:
                cp.start()
        if n == NX - 1:
            for cp in [cp_c] + wcopies(0):
                cp.start()
        cp_xt[n].wait()
        if n == NX - 1:
            for cp in cp_wb:
                cp.wait()
        pks.append(_phi(_dot(wtk, pltpu.bitcast(xt_s[:, n * XC:(n + 1) * XC], BF16))).astype(BF16))
    pk = jnp.concatenate(pks, axis=1)
    xt = pltpu.bitcast(xt_s[...], BF16)
    wtq = wqkv_s[:, 0:512].T[:M]
    wtv = wqkv_s[:, 896:].T
    bwot = bwo_s[...].T
    gw = jnp.broadcast_to(gw_ref[...].reshape(1, M), (16, M))
    vg = _dot(jnp.concatenate([wtv, gw], axis=0), xt)
    v = vg[:M].astype(BF16)
    _st(x_s, (), 0, S, xt.T)
    g_s[...] = 1.0 / (1.0 + jnp.exp(-vg[M:M + 8]))
    cp_wot.start()
    pq = _phi(_dot(wtq, xt)).astype(BF16)

    ri = lax.broadcasted_iota(jnp.int32, (GW, GW), 0)
    ci = lax.broadcasted_iota(jnp.int32, (GW, GW), 1)
    same_head = (ri // DH) == (ci // DH)
    zr = lax.broadcasted_iota(jnp.int32, (16, GW), 0)
    zc = lax.broadcasted_iota(jnp.int32, (16, GW), 1)
    zmask = zr == (zc // DH)
    er = lax.broadcasted_iota(jnp.int32, (GW, S), 0)
    ones = jnp.ones((16, S), BF16)
    kvz = []
    for g in range(G):
        r0, r1 = g * GW, (g + 1) * GW
        r = _dot_nt(jnp.concatenate([v[r0:r1], ones], axis=0), pk[r0:r1])
        kvt = jnp.where(same_head, r[:GW], 0.0)
        zm = jnp.where(zmask, r[GW:], 0.0)
        kvz.append(jnp.concatenate([kvt, zm], axis=0).astype(BF16))
    o_parts = []
    for g in range(G):
        r0, r1 = g * GW, (g + 1) * GW
        nd = _dot(kvz[g], pq[r0:r1])
        rd = 1.0 / (nd[GW:GW + 8] + 1e-6)
        rfull = jnp.where(er < DH, rd[0:1],
                          jnp.where(er < 2 * DH, rd[1:2], jnp.where(er < 3 * DH, rd[2:3], rd[3:4])))
        o_parts.append((nd[:GW] * rfull).astype(BF16))
    bt_s[...] = _dot(bwot, jnp.concatenate(o_parts, axis=0))

    cp_c.wait()

    def proj(j, carry):
        for cp in wcopies(j):
            cp.wait()

        @pl.when(j + 1 < H // 2)
        def _():
            for cp in wcopies(j + 1):
                cp.start()

        for hi in (False, True):
            h = 2 * j + int(hi)
            wq, wk, wv = _half(wq_s[j], hi), _half(wk_s[j], hi), _half(wv_s[j], hi)
            for n in range(NB):
                r0, r1 = n * BQ, (n + 1) * BQ
                c = _ld(c_s, (), r0, r1)
                _st(k_s, (h,), r0, r1, _dot(c, wk).astype(BF16))
                _st(v_s, (h,), r0, r1, _dot(c, wv).astype(BF16))
                q = _dot(_ld(x_s, (), r0, r1), wq) * (D ** -0.5 * LOG2E)
                _st(q_s, (h,), r0, r1, q.astype(BF16))
        return carry

    lax.fori_loop(0, H // 2, proj, 0)

    qi = lax.broadcasted_iota(jnp.int32, (HB, HB), 0)
    kj = lax.broadcasted_iota(jnp.int32, (HB, HB), 1)
    tri = kj <= qi

    def qk(h, i):
        r0, r1 = i * BQ, (i + 1) * BQ
        rm = r0 + HB
        sa = _dot_nt(_ld(q_s, (h,), r0, r1), _ld(k_s, (h,), 0, rm))
        sb = _dot_nt(_ld(q_s, (h,), rm, r1), _ld(k_s, (h,), rm, r1))
        return sa, sb

    def pv(h, i, sa, sb):
        r0, r1 = i * BQ, (i + 1) * BQ
        rm = r0 + HB
        sd = jnp.concatenate([jnp.where(tri, sa[:HB, r0:], MASKED), sa[HB:, r0:]], axis=0)
        sa = sd if i == 0 else jnp.concatenate([sa[:, :r0], sd], axis=1)
        sb = jnp.where(tri, sb, MASKED)
        ma = jnp.max(sa, axis=1, keepdims=True)
        mb = jnp.max(sb, axis=1, keepdims=True)
        m = jnp.concatenate([ma[:HB], jnp.maximum(ma[HB:], mb)], axis=0)
        la = jnp.sum(jnp.exp2(sa - m), axis=1, keepdims=True)
        lb = jnp.sum(jnp.exp2(sb - m[HB:]), axis=1, keepdims=True)
        l = jnp.concatenate([la[:HB], la[HB:] + lb], axis=0)
        lse = m + jnp.log2(l)
        ca = _dot(jnp.exp2(sa - lse).astype(BF16), _ld(v_s, (h,), 0, rm))
        cb = _dot(jnp.exp2(sb - lse[HB:]).astype(BF16), _ld(v_s, (h,), rm, r1))
        ctx = jnp.concatenate([ca[:HB], ca[HB:] + cb], axis=0)
        _st(ctx_s, (h,), r0, r1, ctx.astype(BF16))

    def attend(h, carry):
        pend = []
        for i in ORDER:
            pend.append((i, qk(h, i)))
            if len(pend) > LOOK:
                i0, s0 = pend.pop(0)
                pv(h, i0, *s0)
        for i0, s0 in pend:
            pv(h, i0, *s0)
        return carry

    lax.fori_loop(0, H, attend, 0)

    cp_wot.wait()
    ocopies = []
    for i in range(NB):
        c0, c1 = i * BQ, (i + 1) * BQ
        a = None
        for h in range(H):
            t = _dot_nt(pltpu.bitcast(wot_s[h], BF16), _ld(ctx_s, (h,), c0, c1))
            a = t if a is None else a + t
        g = g_s[0:1, c0:c1]
        out_s[:, c0:c1] = (g * a + (1.0 - g) * bt_s[:, c0:c1]).astype(BF16)
        cp = pltpu.make_async_copy(out_s.at[:, pl.ds(c0, BQ)], out_hbm.at[:, pl.ds(c0, BQ)], osem.at[i])
        cp.start()
        ocopies.append(cp)
    for cp in ocopies:
        cp.wait()


@jax.jit
def pallas_gated_mix__compressed_kv_cla__linear_attn_block__prompt_kernel(
    A_x: jax.Array,
    A_c_kv: jax.Array,
    A_w_q: jax.Array,
    A_w_uk: jax.Array,
    A_w_uv: jax.Array,
    A_w_o: jax.Array,
    B_x: jax.Array,
    B_wqkv: jax.Array,
    B_wo: jax.Array,
    gate_w: jax.Array,
):
    del B_x
    hbm = pl.BlockSpec(memory_space=pl.ANY)
    out_t = pl.pallas_call(
        _kernel,
        out_shape=jax.ShapeDtypeStruct((M, S), BF16),
        in_specs=[hbm] * 8 + [pl.BlockSpec(memory_space=pltpu.VMEM)],
        out_specs=hbm,
        scratch_shapes=[
            pltpu.VMEM((M // 2, S), U32),
            pltpu.VMEM((S // 2, M), U32),
            pltpu.VMEM((S // 2, DC), U32),
            pltpu.VMEM((H // 2, M, D), U32),
            pltpu.VMEM((H // 2, DC, D), U32),
            pltpu.VMEM((H // 2, DC, D), U32),
            pltpu.VMEM((H, M // 2, D), U32),
            pltpu.VMEM((M, 3 * M), BF16),
            pltpu.VMEM((M, M), BF16),
            pltpu.VMEM((H, S // 2, D), U32),
            pltpu.VMEM((H, S // 2, D), U32),
            pltpu.VMEM((H, S // 2, D), U32),
            pltpu.VMEM((H, S // 2, D), U32),
            pltpu.VMEM((M, S), F32),
            pltpu.VMEM((8, S), F32),
            pltpu.VMEM((M, S), BF16),
            pltpu.SemaphoreType.DMA((6 + NX,)),
            pltpu.SemaphoreType.DMA((3 * H // 2,)),
            pltpu.SemaphoreType.DMA((NB,)),
        ],
        compiler_params=pltpu.CompilerParams(vmem_limit_bytes=127 * 2**20),
    )(A_x.reshape(S, M).T, A_c_kv.reshape(S, DC), A_w_q, A_w_uk, A_w_uv,
      A_w_o.transpose(0, 2, 1), B_wqkv, B_wo, gate_w)
    return out_t.T.reshape(1, S, M)
```
